```python
import os as _os
_os.environ.setdefault("JAX_PLATFORMS", "cpu")
import jax
import jax.numpy as jnp

def _softmax(x, axis=-1):
    return jax.nn.softmax(x, axis=axis)
def _gelu(x):
    return jax.nn.gelu(x, approximate=True)
def _silu(x):
    return jax.nn.silu(x)
def _sigmoid(x):
    return jax.nn.sigmoid(x)
def _layernorm(x, axis=-1, eps=1e-5):
    m = jnp.mean(x, axis=axis, keepdims=True)
    v = jnp.var(x, axis=axis, keepdims=True)
    return (x - m) / jnp.sqrt(v + eps)
def _scatter_add(tgt, idx, src, axis=0):
    return tgt.at[idx].add(src)
def _segment_sum(src, seg, n):
    return jax.ops.segment_sum(src, seg, n)
class _Rng:
    def __init__(self, key):
        self._k = key
    def _next(self):
        self._k, sub = jax.random.split(self._k)
        return sub
    def normal(self, shape):
        return jax.random.normal(self._next(), shape, dtype=jnp.bfloat16)
    def randint(self, lo, hi, shape):
        return jax.random.randint(self._next(), shape, lo, hi, dtype=jnp.int32)
    def uniform(self, shape, lo=0.0, hi=1.0):
        return jax.random.uniform(self._next(), shape, jnp.bfloat16, lo, hi)
    def permutation(self, n):
        return jax.random.permutation(self._next(), n)


kernel_name = 'recurrent_scan__ssm_conv_s5__mixer_s_mlp__prompt'

def setup_inputs():
    _rng = _Rng(jax.random.key(int.from_bytes(__import__("os").urandom(4), "little")))
    _w = (lambda a: (lambda t: t.astype(jnp.bfloat16) if jnp.issubdtype(t.dtype, jnp.floating) else t)(jnp.asarray(a)))
    def _A_setup():
        B, S, D = 1, 2048, 640
        P = D
        Lambda_re = -0.5 * jnp.exp((lambda *s: _rng.normal(s) * 0.8)(P))
        Lambda_im = (lambda *s: _rng.normal(s) * 0.8)(P) * 1.0
        B_re = (lambda *s: _rng.normal(s) * 0.8)(P, D) * (D ** -0.5)
        B_im = (lambda *s: _rng.normal(s) * 0.8)(P, D) * (D ** -0.5)
        C_re = (lambda *s: _rng.normal(s) * 0.8)(D, P) * (P ** -0.5)
        C_im = (lambda *s: _rng.normal(s) * 0.8)(D, P) * (P ** -0.5)
        log_dt = (lambda *s: _rng.normal(s) * 0.8)(P) * 0.3 - 2.0
        Dskip = (lambda *s: _rng.normal(s) * 0.8)(D)
        return {
            "x": _w((lambda *s: _rng.normal(s) * 0.05)(B, S, D)),
            "Lambda_re": _w(Lambda_re),
            "Lambda_im": _w(Lambda_im),
            "B_re": _w(B_re),
            "B_im": _w(B_im),
            "C_re": _w(C_re),
            "C_im": _w(C_im),
            "log_dt": _w(log_dt),
            "Dskip": _w(Dskip),
        }
    _A_in = _A_setup()

    def _B_setup():
        B, S, D, F = 1, 2048, 640, 1536
        return {
            "x":  _w((lambda *s: _rng.normal(s) * 0.05)(B, S, D)),
            "w1": _w((lambda *s: _rng.normal(s) * 0.8)(D, D) * (D ** -0.5)),
            "w2": _w((lambda *s: _rng.normal(s) * 0.8)(D, D) * (D ** -0.5)),
            "w3": _w((lambda *s: _rng.normal(s) * 0.8)(D, F) * (D ** -0.5)),
            "w4": _w((lambda *s: _rng.normal(s) * 0.8)(F, D) * (F ** -0.5)),
        }
    _B_in = _B_setup()

    return {
        "A_x": _A_in["x"],
        "A_Lambda_re": _A_in["Lambda_re"],
        "A_Lambda_im": _A_in["Lambda_im"],
        "A_B_re": _A_in["B_re"],
        "A_B_im": _A_in["B_im"],
        "A_C_re": _A_in["C_re"],
        "A_C_im": _A_in["C_im"],
        "A_log_dt": _A_in["log_dt"],
        "A_Dskip": _A_in["Dskip"],
        "B_x": _B_in["x"],
        "B_w1": _B_in["w1"],
        "B_w2": _B_in["w2"],
        "B_w3": _B_in["w3"],
        "B_w4": _B_in["w4"],
    }

def reference(A_x, A_Lambda_re, A_Lambda_im, A_B_re, A_B_im, A_C_re, A_C_im, A_log_dt, A_Dskip, B_x, B_w1, B_w2, B_w3, B_w4):
    def _A_ref(x, Lambda_re, Lambda_im, B_re, B_im, C_re, C_im, log_dt, Dskip):
        Bsz, L, H = x.shape
        Lam = Lambda_re + 1j * Lambda_im
        Bmat = B_re + 1j * B_im
        Cmat = C_re + 1j * C_im
        dt = jnp.exp(log_dt)
        Lam_bar = jnp.exp(dt * Lam)
        B_bar = ((Lam_bar - 1.0) / Lam)[:, None] * Bmat
        Bu = jnp.einsum("bld,pd->blp", x + 0j, B_bar)
        h = jnp.zeros_like(Bu[:, 0, :])
        hs = []
        for t in range(L):
            h = Lam_bar[None, :] * h + Bu[:, t, :]
            hs.append(h)
        hseq = jnp.stack(hs, 1)
        y = 2.0 * jnp.einsum("blp,dp->bld", hseq, Cmat).real + x * Dskip[None, None, :]
        return y

    def _B_ref(x, w1, w2, w3, w4):
        B, S, D = x.shape
        h = _gelu(_layernorm(x, axis=-1) @ w1)
        c = D // 4
        g0 = jnp.pad(h[:, :, 0*c:1*c], ((0, 0), (1, 0), (0, 0)))[:, :S, :]
        g1 = jnp.pad(h[:, :, 1*c:2*c], ((0, 0), (0, 1), (0, 0)))[:, 1:, :]
        g2 = jnp.pad(h[:, :, 2*c:3*c], ((0, 0), (2, 0), (0, 0)))[:, :S, :]
        g3 = jnp.pad(h[:, :, 3*c:   ], ((0, 0), (0, 2), (0, 0)))[:, 2:, :]
        hs = jnp.concatenate([g0, g1, g2, g3], axis=-1) @ w2
        x1 = x + hs
        h2 = _gelu(_layernorm(x1, axis=-1) @ w3) @ w4
        return x1 + h2

    x = A_x
    xn = _layernorm(x, axis=-1)
    s = _A_ref(xn, A_Lambda_re, A_Lambda_im, A_B_re, A_B_im, A_C_re, A_C_im, A_log_dt, A_Dskip)
    g = _silu(_B_ref(xn, B_w1, B_w2, B_w3, B_w4))
    return x + s * g
```

```python
import functools
import jax
import jax.numpy as jnp
import jax.experimental.pallas as pl
import jax.experimental.pallas.tpu as pltpu

S = 2048
D = 640
P = 640
F = 1536
R = 256
NB = S // R
NC = 8
T = R // NC
PIT = T + 1
NT = P // 128
HALO = 16
EPS = 1e-5


def _ln(x):
    m = jnp.mean(x, axis=-1, keepdims=True)
    xc = x - m
    v = jnp.mean(xc * xc, axis=-1, keepdims=True)
    return xc * jax.lax.rsqrt(v + EPS)


def _cmul(ar, ai, br, bi):
    return ar * br - ai * bi, ar * bi + ai * br


def _kernel(x_ref, xnext_ref, lre_ref, lim_ref, ldt_ref, dsk_ref, bre_hbm, bim_hbm, cre_hbm, cim_hbm,
            w1_hbm, w2_hbm, w3_hbm, w4_hbm, o_ref,
            cre_ref, cim_ref, w1_ref, w2_ref, w3_ref, w4_ref, sems,
            bt_ref, ct_ref, par_ref, st_ref, xp_ref, yp_ref, h1_ref,
            xn_buf, z_buf, xq_buf):
    i = pl.program_id(0)
    cur = i % 2
    nxt = 1 - cur
    copies = [pltpu.make_async_copy(src, dst, sems.at[k]) for k, (src, dst) in enumerate((
        (bre_hbm, bt_ref.at[0:P]), (bim_hbm, bt_ref.at[P:2 * P]), (w1_hbm, w1_ref), (w2_hbm, w2_ref),
        (cre_hbm, cre_ref), (cim_hbm, cim_ref), (w3_hbm, w3_ref), (w4_hbm, w4_ref)))]
    cp_bre, cp_bim, cp_w1, cp_w2, cp_cre, cp_cim, cp_w3, cp_w4 = copies

    def front(src_ref, slot):
        xn = _ln(src_ref[...].astype(jnp.float32)).astype(jnp.bfloat16).astype(jnp.float32)
        xn_buf[slot] = xn
        z = _ln(xn).astype(jnp.bfloat16)
        z_buf[slot] = z
        for j in range(NT):
            for c in range(NC):
                xp_ref[j, c * PIT:c * PIT + T, :] = xn[c * T:(c + 1) * T, 128 * j:128 * (j + 1)]
        xq_buf[slot] = jnp.concatenate(
            [jnp.concatenate([xp_ref[j, pl.ds(t, NC, stride=PIT), :] for j in range(NT)], axis=1)
             for t in range(T)], axis=0).astype(jnp.bfloat16)
        return z[0:HALO]

    def body(first):
        if first:
            for cp in copies:
                cp.start()
            lre = lre_ref[...].astype(jnp.float32).reshape(1, P)
            lim = lim_ref[...].astype(jnp.float32).reshape(1, P)
            dt = jnp.exp(ldt_ref[...].astype(jnp.float32).reshape(1, P)).astype(jnp.bfloat16).astype(jnp.float32)
            mag = jnp.exp(dt * lre)
            ang = dt * lim
            a_r = mag * jnp.cos(ang)
            a_i = mag * jnp.sin(ang)
            nr = a_r - 1.0
            ni = a_i
            den = lre * lre + lim * lim
            cr = (nr * lre + ni * lim) / den
            ci = (ni * lre - nr * lim) / den
            pr, pi = a_r, a_i
            t = 1
            while t < T:
                pr, pi = _cmul(pr, pi, pr, pi)
                t *= 2
            par_ref[0:1, :] = a_r
            par_ref[1:2, :] = a_i
            par_ref[2:3, :] = pr
            par_ref[3:4, :] = pi
            p2r, p2i = _cmul(pr, pi, pr, pi)
            par_ref[4:5, :] = p2r
            par_ref[5:6, :] = p2i
            p4r, p4i = _cmul(p2r, p2i, p2r, p2i)
            par_ref[6:7, :] = p4r
            par_ref[7:8, :] = p4i
            st_ref[...] = jnp.zeros_like(st_ref)
            h1_ref[0:8, :] = jnp.zeros((8, D), jnp.float32)
            front(x_ref, 0)
            cp_bre.wait()
            cp_bim.wait()

        u = jax.lax.dot_general(xq_buf[cur], bt_ref[...], (((1,), (1,)), ((), ())),
                                preferred_element_type=jnp.float32)

        zh = front(xnext_ref, nxt)

        z = jnp.concatenate([z_buf[cur], zh], axis=0)
        if first:
            cp_w1.wait()
        h1 = jax.nn.gelu(jnp.dot(z, w1_ref[...], preferred_element_type=jnp.float32), approximate=True)

        ar = jnp.broadcast_to(par_ref[0:1, :], (NC, P))
        ai = jnp.broadcast_to(par_ref[1:2, :], (NC, P))
        hr = jnp.zeros((NC, P), jnp.float32)
        hi = jnp.zeros((NC, P), jnp.float32)
        for t in range(T):
            ur = u[t * NC:(t + 1) * NC, 0:P]
            ui = u[t * NC:(t + 1) * NC, P:2 * P]
            hr, hi = ar * hr - ai * hi + ur, ar * hi + ai * hr + ui
        sub = jax.lax.broadcasted_iota(jnp.int32, (NC, P), 0)
        fr = jnp.where(sub == 0, st_ref[0:NC, :], pltpu.roll(hr, 1, 0))
        fi = jnp.where(sub == 0, st_ref[NC:2 * NC, :], pltpu.roll(hi, 1, 0))
        for k, row in ((1, 2), (2, 4), (4, 6)):
            kr = par_ref[row:row + 1, :]
            ki = par_ref[row + 1:row + 2, :]
            sr = jnp.where(sub >= k, pltpu.roll(fr, k, 0), 0.0)
            si = jnp.where(sub >= k, pltpu.roll(fi, k, 0), 0.0)
            fr, fi = fr + kr * sr - ki * si, fi + kr * si + ki * sr
        Ar = par_ref[2:3, :]
        Ai = par_ref[3:4, :]
        gr = Ar * fr - Ai * fi + hr
        gi = Ar * fi + Ai * fr + hi
        st_ref[0:NC, :] = pltpu.roll(gr, 1, 0)
        st_ref[NC:2 * NC, :] = pltpu.roll(gi, 1, 0)
        hr, hi = fr, fi
        hs = []
        for t in range(T):
            ur = u[t * NC:(t + 1) * NC, 0:P]
            ui = u[t * NC:(t + 1) * NC, P:2 * P]
            hr, hi = ar * hr - ai * hi + ur, ar * hi + ai * hr + ui
            hs.append(jnp.concatenate([hr, hi], axis=1))
        hh = jnp.concatenate(hs, axis=0).astype(jnp.bfloat16)

        h1_ref[8:8 + R, :] = h1[0:R]
        h1_ref[8 + R:16 + R, :] = jnp.where(i < NB - 1, h1[R:R + 8], 0.0)
        lane = jax.lax.broadcasted_iota(jnp.int32, (R, 128), 1)

        def sh(s_, j):
            return h1_ref[8 - s_:8 - s_ + R, 128 * j:128 * (j + 1)]
        g = jnp.concatenate([
            sh(1, 0),
            jnp.where(lane < 32, sh(1, 1), sh(-1, 1)),
            jnp.where(lane < 64, sh(-1, 2), sh(2, 2)),
            jnp.where(lane < 96, sh(2, 3), sh(-2, 3)),
            sh(-2, 4)], axis=1).astype(jnp.bfloat16)
        h1_ref[0:8, :] = h1[R - 8:R]
        if first:
            cp_w2.wait()
        xn = xn_buf[cur]
        x1 = xn + jnp.dot(g, w2_ref[...], preferred_element_type=jnp.float32)
        z2 = _ln(x1).astype(jnp.bfloat16)

        if first:
            cp_cre.wait()
            cp_cim.wait()
            c_r = cre_ref[...].astype(jnp.float32)
            c_i = cim_ref[...].astype(jnp.float32)
            ct_ref[:, 0:P] = (c_r * (2.0 * cr) - c_i * (2.0 * ci)).astype(jnp.bfloat16)
            ct_ref[:, P:2 * P] = (c_r * (-2.0 * ci) - c_i * (2.0 * cr)).astype(jnp.bfloat16)
        yp = jax.lax.dot_general(hh, ct_ref[...], (((1,), (1,)), ((), ())),
                                 preferred_element_type=jnp.float32)
        for t in range(T):
            for j in range(NT):
                yp_ref[j, pl.ds(t, NC, stride=PIT), :] = yp[t * NC:(t + 1) * NC, 128 * j:128 * (j + 1)]
        y = jnp.concatenate(
            [jnp.concatenate([yp_ref[j, c * PIT:c * PIT + T, :] for j in range(NT)], axis=1)
             for c in range(NC)], axis=0)
        s = y + xn * dsk_ref[...].astype(jnp.float32).reshape(1, D)

        if first:
            cp_w3.wait()
        h2 = jax.nn.gelu(jnp.dot(z2, w3_ref[...], preferred_element_type=jnp.float32), approximate=True)
        if first:
            cp_w4.wait()
        m = x1 + jnp.dot(h2.astype(jnp.bfloat16), w4_ref[...], preferred_element_type=jnp.float32)
        o_ref[...] = x_ref[...].astype(jnp.float32) + s * jax.nn.silu(m)

    @pl.when(i == 0)
    def _():
        body(True)

    @pl.when(i > 0)
    def _():
        body(False)


@jax.jit
def pallas_recurrent_scan__ssm_conv_s5__mixer_s_mlp__prompt_kernel(
    A_x, A_Lambda_re, A_Lambda_im, A_B_re, A_B_im, A_C_re, A_C_im, A_log_dt, A_Dskip,
    B_x, B_w1, B_w2, B_w3, B_w4,
):
    x = A_x.reshape(S, D)
    vec = pl.BlockSpec((P,), lambda i: (0,))
    hbm = pl.BlockSpec(memory_space=pl.ANY)
    out = pl.pallas_call(
        _kernel,
        grid=(NB,),
        in_specs=[pl.BlockSpec((R, D), lambda i: (i, 0)),
                  pl.BlockSpec((R, D), lambda i: (jnp.minimum(i + 1, NB - 1), 0)),
                  vec, vec, vec, vec,
                  hbm, hbm, hbm, hbm, hbm, hbm, hbm, hbm],
        out_specs=pl.BlockSpec((R, D), lambda i: (i, 0)),
        out_shape=jax.ShapeDtypeStruct((S, D), jnp.float32),
        scratch_shapes=[
            pltpu.VMEM((D, P), jnp.bfloat16),
            pltpu.VMEM((D, P), jnp.bfloat16),
            pltpu.VMEM((D, D), jnp.bfloat16),
            pltpu.VMEM((D, D), jnp.bfloat16),
            pltpu.VMEM((D, F), jnp.bfloat16),
            pltpu.VMEM((F, D), jnp.bfloat16),
            pltpu.SemaphoreType.DMA((8,)),
            pltpu.VMEM((2 * P, D), jnp.bfloat16),
            pltpu.VMEM((D, 2 * P), jnp.bfloat16),
            pltpu.VMEM((8, P), jnp.float32),
            pltpu.VMEM((2 * NC, P), jnp.float32),
            pltpu.VMEM((NT, NC * PIT, 128), jnp.float32),
            pltpu.VMEM((NT, NC * PIT, 128), jnp.float32),
            pltpu.VMEM((R + 16, D), jnp.float32),
            pltpu.VMEM((2, R, D), jnp.float32),
            pltpu.VMEM((2, R, D), jnp.bfloat16),
            pltpu.VMEM((2, R, D), jnp.bfloat16),
        ],
        compiler_params=pltpu.CompilerParams(
            dimension_semantics=("arbitrary",),
            vmem_limit_bytes=100 * 1024 * 1024),
    )(x, x, A_Lambda_re, A_Lambda_im, A_log_dt, A_Dskip, A_B_re, A_B_im, A_C_re, A_C_im, B_w1, B_w2, B_w3, B_w4)
    return out.reshape(1, S, D)
```

```python
import jax
import jax.numpy as jnp
import jax.experimental.pallas as pl
import jax.experimental.pallas.tpu as pltpu

S = 2048
D = 640
P = 640
F = 1536
R = 256
NB = S // R
NC = 8
T = R // NC
PIT = T + 1
NT = P // 128
HALO = 16
EPS = 1e-5
_NT_DIMS = (((1,), (1,)), ((), ()))


def _ln(x):
    m = jnp.mean(x, axis=-1, keepdims=True)
    xc = x - m
    v = jnp.mean(xc * xc, axis=-1, keepdims=True)
    return xc * jax.lax.rsqrt(v + EPS)


def _cmul(ar, ai, br, bi):
    return ar * br - ai * bi, ar * bi + ai * br


def _dot(a, b):
    return jnp.dot(a, b, preferred_element_type=jnp.float32)


def _dot_nt(a, b):
    return jax.lax.dot_general(a, b, _NT_DIMS, preferred_element_type=jnp.float32)


def _kernel(x_hbm, lre_hbm, lim_hbm, ldt_hbm, dsk_hbm,
            bre_hbm, bim_hbm, cre_hbm, cim_hbm, w1_hbm, w2_hbm, w3_hbm, w4_hbm, o_hbm,
            x_ref, lre_ref, lim_ref, ldt_ref, dsk_ref,
            cre_ref, cim_ref, w1_ref, w2_ref, w3_ref, w4_ref, wsem, vsem, xsem, osem, hsem,
            bt_ref, ct_ref, par_ref, st_ref, xp_ref, sp_ref, h1_ref, x1_ref, z2_ref, o_buf):
    wcp = [pltpu.make_async_copy(src, dst, wsem.at[k]) for k, (src, dst) in enumerate((
        (w1_hbm, w1_ref), (bre_hbm, bt_ref.at[0:P]), (bim_hbm, bt_ref.at[P:2 * P]), (w2_hbm, w2_ref),
        (cre_hbm, cre_ref), (cim_hbm, cim_ref), (w3_hbm, w3_ref), (w4_hbm, w4_ref)))]
    cp_w1, cp_bre, cp_bim, cp_w2, cp_cre, cp_cim, cp_w3, cp_w4 = wcp
    vcp = [pltpu.make_async_copy(src, dst, vsem.at[k]) for k, (src, dst) in enumerate((
        (lre_hbm, lre_ref), (lim_hbm, lim_ref), (ldt_hbm, ldt_ref), (dsk_hbm, dsk_ref)))]
    xcp = [pltpu.make_async_copy(x_hbm.at[k * R:(k + 1) * R], x_ref.at[k * R:(k + 1) * R], xsem.at[k])
           for k in range(NB)]

    def ocp(blk, slot):
        return pltpu.make_async_copy(o_buf.at[slot], o_hbm.at[pl.ds(pl.multiple_of(blk * R, R), R)],
                                     osem.at[slot])

    def ocp_h(blk, slot, q):
        H = R // 2
        return pltpu.make_async_copy(o_buf.at[slot, q * H:(q + 1) * H],
                                     o_hbm.at[pl.ds(pl.multiple_of(blk * R + q * H, H), H)],
                                     hsem.at[2 * slot + q])

    def params():
        lre = lre_ref[...].astype(jnp.float32).reshape(1, P)
        lim = lim_ref[...].astype(jnp.float32).reshape(1, P)
        dt = jnp.exp(ldt_ref[...].astype(jnp.float32).reshape(1, P))
        dt = dt.astype(jnp.bfloat16).astype(jnp.float32)
        mag = jnp.exp(dt * lre)
        ang = dt * lim
        a_r = mag * jnp.cos(ang)
        a_i = mag * jnp.sin(ang)
        nr = a_r - 1.0
        ni = a_i
        den = lre * lre + lim * lim
        cr = (nr * lre + ni * lim) / den
        ci = (ni * lre - nr * lim) / den
        pr, pi = a_r, a_i
        t = 1
        while t < T:
            pr, pi = _cmul(pr, pi, pr, pi)
            t *= 2
        par_ref[0:1, :] = a_r
        par_ref[1:2, :] = a_i
        par_ref[2:3, :] = pr
        par_ref[3:4, :] = pi
        p2r, p2i = _cmul(pr, pi, pr, pi)
        par_ref[4:5, :] = p2r
        par_ref[5:6, :] = p2i
        p4r, p4i = _cmul(p2r, p2i, p2r, p2i)
        par_ref[6:7, :] = p4r
        par_ref[7:8, :] = p4i
        st_ref[...] = jnp.zeros_like(st_ref)
        h1_ref[0:8, :] = jnp.zeros((8, D), jnp.float32)
        return cr, ci

    def front(i, slot):
        r0 = pl.multiple_of(i * R, R)
        rh = pl.multiple_of(jnp.minimum(r0 + R, S - HALO), HALO)
        xn = _ln(x_ref[pl.ds(r0, R), :].astype(jnp.float32)).astype(jnp.bfloat16).astype(jnp.float32)
        xhn = _ln(x_ref[pl.ds(rh, HALO), :].astype(jnp.float32)).astype(jnp.bfloat16).astype(jnp.float32)
        z = jnp.concatenate([_ln(xn), _ln(xhn)], axis=0).astype(jnp.bfloat16)
        for j in range(NT):
            for c in range(NC):
                xp_ref[slot, j, c * PIT:c * PIT + T, :] = xn[c * T:(c + 1) * T, 128 * j:128 * (j + 1)]
        xq = jnp.concatenate(
            [jnp.concatenate([xp_ref[slot, j, pl.ds(t, NC, stride=PIT), :] for j in range(NT)], axis=1)
             for t in range(T)], axis=0)
        return xn, z, xq

    def mix1(z):
        return jax.nn.gelu(_dot(z, w1_ref[...]), approximate=True)

    def scan(u):
        ar = jnp.broadcast_to(par_ref[0:1, :], (NC, P))
        ai = jnp.broadcast_to(par_ref[1:2, :], (NC, P))
        hr = jnp.zeros((NC, P), jnp.float32)
        hi = jnp.zeros((NC, P), jnp.float32)
        for t in range(T):
            ur = u[t * NC:(t + 1) * NC, 0:P]
            ui = u[t * NC:(t + 1) * NC, P:2 * P]
            hr, hi = ar * hr - ai * hi + ur, ar * hi + ai * hr + ui
        sub = jax.lax.broadcasted_iota(jnp.int32, (NC, P), 0)
        fr = jnp.where(sub == 0, st_ref[0:NC, :], pltpu.roll(hr, 1, 0))
        fi = jnp.where(sub == 0, st_ref[NC:2 * NC, :], pltpu.roll(hi, 1, 0))
        for k, row in ((1, 2), (2, 4), (4, 6)):
            kr = par_ref[row:row + 1, :]
            ki = par_ref[row + 1:row + 2, :]
            sr = jnp.where(sub >= k, pltpu.roll(fr, k, 0), 0.0)
            si = jnp.where(sub >= k, pltpu.roll(fi, k, 0), 0.0)
            fr, fi = fr + kr * sr - ki * si, fi + kr * si + ki * sr
        Ar = par_ref[2:3, :]
        Ai = par_ref[3:4, :]
        gr = Ar * fr - Ai * fi + hr
        gi = Ar * fi + Ai * fr + hi
        st_ref[0:NC, :] = pltpu.roll(gr, 1, 0)
        st_ref[NC:2 * NC, :] = pltpu.roll(gi, 1, 0)
        hr, hi = fr, fi
        hs = []
        for t in range(T):
            ur = u[t * NC:(t + 1) * NC, 0:P]
            ui = u[t * NC:(t + 1) * NC, P:2 * P]
            hr, hi = ar * hr - ai * hi + ur, ar * hi + ai * hr + ui
            hs.append(jnp.concatenate([hr, hi], axis=1))
        return jnp.concatenate(hs, axis=0).astype(jnp.bfloat16)

    def shift(i, h1):
        h1_ref[8:8 + R, :] = h1[0:R]
        h1_ref[8 + R:16 + R, :] = jnp.where(i < NB - 1, h1[R:R + 8], 0.0)
        lane = jax.lax.broadcasted_iota(jnp.int32, (R, 128), 1)

        def sh(s_, j):
            return h1_ref[8 - s_:8 - s_ + R, 128 * j:128 * (j + 1)]
        g = jnp.concatenate([
            sh(1, 0),
            jnp.where(lane < 32, sh(1, 1), sh(-1, 1)),
            jnp.where(lane < 64, sh(-1, 2), sh(2, 2)),
            jnp.where(lane < 96, sh(2, 3), sh(-2, 3)),
            sh(-2, 4)], axis=1).astype(jnp.bfloat16)
        h1_ref[0:8, :] = h1[R - 8:R]
        return g

    def back(par, xn, xq, g, hh):
        x1 = xn + _dot(g, w2_ref[...])
        x1_ref[par] = x1
        z2_ref[par] = _ln(x1).astype(jnp.bfloat16)
        sq = _dot_nt(hh, ct_ref[...]) + xq * dsk_ref[...].astype(jnp.float32).reshape(1, D)
        for t in range(T):
            for j in range(NT):
                sp_ref[par, j, pl.ds(t, NC, stride=PIT), :] = sq[t * NC:(t + 1) * NC, 128 * j:128 * (j + 1)]

    def phase1(blk, par):
        h2 = jax.nn.gelu(_dot(z2_ref[par], w3_ref[...]), approximate=True).astype(jnp.bfloat16)
        s = jnp.concatenate(
            [jnp.concatenate([sp_ref[par, j, c * PIT:c * PIT + T, :] for j in range(NT)], axis=1)
             for c in range(NC)], axis=0)
        m = x1_ref[par] + _dot(h2, w4_ref[...])
        xb = x_ref[pl.ds(pl.multiple_of(blk * R, R), R), :].astype(jnp.float32)
        o_buf[par] = xb + s * jax.nn.silu(m)
        ocp(blk, par).start()

    def phase1_split(blk, par):
        H = R // 2
        h2 = jax.nn.gelu(_dot(z2_ref[par], w3_ref[...]), approximate=True).astype(jnp.bfloat16)
        for q in range(2):
            s = jnp.concatenate(
                [jnp.concatenate([sp_ref[par, j, c * PIT:c * PIT + T, :] for j in range(NT)], axis=1)
                 for c in range(q * NC // 2, (q + 1) * NC // 2)], axis=0)
            m = x1_ref[par, q * H:(q + 1) * H, :] + _dot(h2[q * H:(q + 1) * H], w4_ref[...])
            xb = x_ref[pl.ds(pl.multiple_of(blk * R + q * H, H), H), :].astype(jnp.float32)
            o_buf[par, q * H:(q + 1) * H, :] = xb + s * jax.nn.silu(m)
            ocp_h(blk, par, q).start()

    def make_ct(cr, ci):
        c_r = cre_ref[...].astype(jnp.float32)
        c_i = cim_ref[...].astype(jnp.float32)
        ct_ref[:, 0:P] = (c_r * (2.0 * cr) - c_i * (2.0 * ci)).astype(jnp.bfloat16)
        ct_ref[:, P:2 * P] = (c_r * (-2.0 * ci) - c_i * (2.0 * cr)).astype(jnp.bfloat16)

    for cp in vcp:
        cp.start()
    xcp[0].start()
    xcp[1].start()
    xcp[2].start()
    for cp in vcp:
        cp.wait()
    for cp in wcp:
        cp.start()
    for k in range(3, NB):
        xcp[k].start()

    cr, ci = params()
    xcp[0].wait()
    xcp[1].wait()
    xcp[2].wait()
    xn0, z0, xq0 = front(0, 0)
    cp_w1.wait()
    h10 = mix1(z0)
    xn1, z1, xq1 = front(1, 1)
    h11 = mix1(z1)
    g0 = shift(0, h10)
    g1 = shift(1, h11)
    cp_bre.wait()
    cp_bim.wait()
    u0 = _dot_nt(xq0.astype(jnp.bfloat16), bt_ref[...])
    u1 = _dot_nt(xq1.astype(jnp.bfloat16), bt_ref[...])
    hh0 = scan(u0)
    hh1 = scan(u1)
    cp_w2.wait()
    cp_cre.wait()
    cp_cim.wait()
    make_ct(cr, ci)
    back(0, xn0, xq0, g0, hh0)
    back(1, xn1, xq1, g1, hh1)
    cp_w3.wait()
    cp_w4.wait()

    def main_body(i, carry):
        par = i % 2

        @pl.when(i >= 4)
        def _():
            ocp(i - 4, par).wait()

        @pl.when(i < NB - 1)
        def _():
            nx = pl.ds(pl.multiple_of((i + 1) * R, R), R)
            pltpu.make_async_copy(x_hbm.at[nx], x_ref.at[nx], xsem.at[i + 1]).wait()
        phase1(i - 2, par)
        xn, z, xq = front(i, 0)
        u = _dot_nt(xq.astype(jnp.bfloat16), bt_ref[...])
        h1 = mix1(z)
        hh = scan(u)
        g = shift(i, h1)
        back(par, xn, xq, g, hh)
        return carry

    jax.lax.fori_loop(2, NB, main_body, 0)

    def tail_body(i, carry):
        par = i % 2
        ocp(i - 4, par).wait()
        phase1_split(i - 2, par)
        return carry

    jax.lax.fori_loop(NB, NB + 2, tail_body, 0)
    for q in range(2):
        ocp_h(NB - 2, 0, q).wait()
        ocp_h(NB - 1, 1, q).wait()


@jax.jit
def pallas_recurrent_scan__ssm_conv_s5__mixer_s_mlp__prompt_kernel(
    A_x, A_Lambda_re, A_Lambda_im, A_B_re, A_B_im, A_C_re, A_C_im, A_log_dt, A_Dskip,
    B_x, B_w1, B_w2, B_w3, B_w4,
):
    x = A_x.reshape(S, D)
    hbm = pl.BlockSpec(memory_space=pl.ANY)
    out = pl.pallas_call(
        _kernel,
        in_specs=[hbm] * 13,
        out_specs=hbm,
        out_shape=jax.ShapeDtypeStruct((S, D), jnp.float32),
        scratch_shapes=[
            pltpu.VMEM((S, D), jnp.bfloat16),
            pltpu.VMEM((P,), jnp.bfloat16),
            pltpu.VMEM((P,), jnp.bfloat16),
            pltpu.VMEM((P,), jnp.bfloat16),
            pltpu.VMEM((D,), jnp.bfloat16),
            pltpu.VMEM((D, P), jnp.bfloat16),
            pltpu.VMEM((D, P), jnp.bfloat16),
            pltpu.VMEM((D, D), jnp.bfloat16),
            pltpu.VMEM((D, D), jnp.bfloat16),
            pltpu.VMEM((D, F), jnp.bfloat16),
            pltpu.VMEM((F, D), jnp.bfloat16),
            pltpu.SemaphoreType.DMA((8,)),
            pltpu.SemaphoreType.DMA((4,)),
            pltpu.SemaphoreType.DMA((NB,)),
            pltpu.SemaphoreType.DMA((2,)),
            pltpu.SemaphoreType.DMA((4,)),
            pltpu.VMEM((2 * P, D), jnp.bfloat16),
            pltpu.VMEM((D, 2 * P), jnp.bfloat16),
            pltpu.VMEM((8, P), jnp.float32),
            pltpu.VMEM((2 * NC, P), jnp.float32),
            pltpu.VMEM((2, NT, NC * PIT, 128), jnp.float32),
            pltpu.VMEM((2, NT, NC * PIT, 128), jnp.float32),
            pltpu.VMEM((R + 16, D), jnp.float32),
            pltpu.VMEM((2, R, D), jnp.float32),
            pltpu.VMEM((2, R, D), jnp.bfloat16),
            pltpu.VMEM((2, R, D), jnp.float32),
        ],
        compiler_params=pltpu.CompilerParams(vmem_limit_bytes=100 * 1024 * 1024),
    )(x, A_Lambda_re, A_Lambda_im, A_log_dt, A_Dskip,
      A_B_re, A_B_im, A_C_re, A_C_im, B_w1, B_w2, B_w3, B_w4)
    return out.reshape(1, S, D)
```
